```python
import jax
import jax.numpy as jnp

def _softmax(x, axis=-1):
    return jax.nn.softmax(x, axis=axis)

def _gelu(x):
    return jax.nn.gelu(x, approximate=True)

def _silu(x):
    return jax.nn.silu(x)

def _sigmoid(x):
    return jax.nn.sigmoid(x)

def _layernorm(x, axis=-1, eps=1e-05):
    m = jnp.mean(x, axis=axis, keepdims=True)
    v = jnp.var(x, axis=axis, keepdims=True)
    return (x - m) / jnp.sqrt(v + eps)

def _scatter_add(tgt, idx, src, axis=0):
    return tgt.at[idx].add(src)

def _segment_sum(src, seg, n):
    return jax.ops.segment_sum(src, seg, n)

class _Rng:

    def __init__(self, key):
        self._k = key

    def _next(self):
        self._k, sub = jax.random.split(self._k)
        return sub

    def normal(self, shape):
        return jax.random.normal(self._next(), shape, dtype=jnp.bfloat16)

    def randint(self, lo, hi, shape):
        return jax.random.randint(self._next(), shape, lo, hi, dtype=jnp.int32)

    def uniform(self, shape, lo=0.0, hi=1.0):
        return jax.random.uniform(self._next(), shape, jnp.bfloat16, lo, hi)

    def permutation(self, n):
        return jax.random.permutation(self._next(), n)
kernel_name = 'adaLN_cond__memory_aug_recurrent_mem_tr__dense_activation_gelu__prompt'

def setup_inputs():
    _rng = _Rng(jax.random.key(int.from_bytes(__import__("os").urandom(4), "little")))
    _w = lambda a: (lambda t: t.astype(jnp.bfloat16) if jnp.issubdtype(t.dtype, jnp.floating) else t)(jnp.asarray(a))

    def _A_setup():
        B, S, Dm = (1, 2048, 1024)
        H, Dh = (32, 128)
        M, seg = (8, 32)
        seg = min(seg, S)
        S = S // seg * seg
        return {'x': _w((lambda *s: _rng.normal(s) * 0.05)(B, S, Dm)), 'mem0': _w((lambda *s: _rng.normal(s) * 0.05)(B, M, Dm)), 'Wq': _w((lambda *s: _rng.normal(s) * 0.05)(Dm, H, Dh) * Dm ** (-0.5)), 'Wk': _w((lambda *s: _rng.normal(s) * 0.05)(Dm, H, Dh) * Dm ** (-0.5)), 'Wv': _w((lambda *s: _rng.normal(s) * 0.05)(Dm, H, Dh) * Dm ** (-0.5)), 'Wo': _w((lambda *s: _rng.normal(s) * 0.05)(H, Dh, Dm) * (H * Dh) ** (-0.5)), 'seg_len': seg}
    _A_in = _A_setup()

    def _B_setup():
        B, S, D, F = (1, 2048, 1024, 3584)
        return {'x': _w((lambda *s: _rng.normal(s) * 0.05)(B, S, D)), 'w1': _w((lambda *s: _rng.normal(s) * 0.05)(D, F) * D ** (-0.5)), 'b1': _w((lambda *s: _rng.normal(s) * 0.05)(F) * 0.01), 'w2': _w((lambda *s: _rng.normal(s) * 0.05)(F, D) * F ** (-0.5)), 'b2': _w((lambda *s: _rng.normal(s) * 0.05)(D) * 0.01)}
    _B_in = _B_setup()
    return {'A_x': _A_in['x'], 'A_mem0': _A_in['mem0'], 'A_Wq': _A_in['Wq'], 'A_Wk': _A_in['Wk'], 'A_Wv': _A_in['Wv'], 'A_Wo': _A_in['Wo'], 'A_seg_len': _A_in['seg_len'], 'B_x': _B_in['x'], 'B_w1': _B_in['w1'], 'B_b1': _B_in['b1'], 'B_w2': _B_in['w2'], 'B_b2': _B_in['b2'], 'c': _w((lambda *s: _rng.normal(s) * 0.05)(1, 1024)), 'w_mod': _w((lambda *s: _rng.normal(s) * 0.05)(1024, 6 * 1024) * 1024 ** (-0.5))}

def reference(A_x, A_mem0, A_Wq, A_Wk, A_Wv, A_Wo, A_seg_len, B_x, B_w1, B_b1, B_w2, B_b2, c, w_mod):

    def _A_ref(x, mem0, Wq, Wk, Wv, Wo, seg_len):
        B, S, Dm = x.shape
        H, Dh = (Wq.shape[1], Wq.shape[2])
        M = mem0.shape[1]
        scale = Dh ** (-0.5)
        n_seg = S // seg_len
        L = M + seg_len
        idx = jnp.arange(L)
        mask = (idx[:, None] < M) | (idx[:, None] >= idx[None, :])
        mem = mem0
        outs = []
        for s in range(n_seg):
            xs = x[:, s * seg_len:(s + 1) * seg_len, :].copy()
            h = jnp.concatenate([mem, xs], axis=1)
            q = jnp.einsum('btd,dhe->bhte', h, Wq)
            k = jnp.einsum('btd,dhe->bhte', h, Wk)
            v = jnp.einsum('btd,dhe->bhte', h, Wv)
            scores = jnp.einsum('bhqe,bhke->bhqk', q, k) * scale
            scores = jnp.where(mask[None, None], scores, -1000000000.0)
            p = _softmax(scores, axis=-1)
            o = jnp.einsum('bhqk,bhke->bhqe', p, v)
            o = jnp.einsum('bhte,hed->btd', o, Wo)
            mem = o[:, :M, :].copy()
            outs.append(o[:, M:, :])
        return jnp.concatenate(outs, axis=1)

    def _B_ref(x, w1, b1, w2, b2):
        h = jnp.einsum('bsd,df->bsf', x, w1) + b1
        h = _gelu(h)
        return jnp.einsum('bsf,fd->bsd', h, w2) + b2
    x = A_x
    mod = (_silu(c) @ w_mod).reshape(c.shape[0], 6, 1, -1)
    sa, ca, ga, sb, cb, gb = (mod[:, 0].copy(), mod[:, 1].copy(), mod[:, 2].copy(), mod[:, 3].copy(), mod[:, 4].copy(), mod[:, 5].copy())
    h = _layernorm(x, axis=-1) * (1 + ca) + sa
    x = x + ga * _A_ref(h, A_mem0, A_Wq, A_Wk, A_Wv, A_Wo, A_seg_len)
    h = _layernorm(x, axis=-1) * (1 + cb) + sb
    x = x + gb * _B_ref(h, B_w1, B_b1, B_w2, B_b2)
    return x
```

```python
import functools

import jax
import jax.numpy as jnp
import numpy as np
from jax import lax
import jax.experimental.pallas as pl
import jax.experimental.pallas.tpu as pltpu

S, DM, H, DH, M, SEG, FF = 2048, 1024, 32, 128, 8, 32, 3584
NSEG = S // SEG
TOK = 24
LEAD = S - NSEG * TOK
RING = 576
ROFF = (-LEAD) % TOK
NIT = NSEG // 2
BLK = 2 * TOK
HC = 8
EPS = 1e-5
F32, BF16, U32 = jnp.float32, jnp.bfloat16, jnp.uint32


def _ln_mod(x, scale, shift):
    m = jnp.mean(x, axis=-1, keepdims=True)
    xc = x - m
    v = jnp.mean(xc * xc, axis=-1, keepdims=True)
    return xc * lax.rsqrt(v + EPS) * (1.0 + scale) + shift


def _gelu(x):
    c = float(np.sqrt(2.0 / np.pi))
    return 0.5 * x * (1.0 + jnp.tanh(c * (x + 0.044715 * (x * x * x))))


def _w(ref_val):
    return pltpu.bitcast(ref_val, BF16)


def _dot(a, b):
    return jnp.dot(a, b, preferred_element_type=F32)


def _kernel(x_hbm, mem0_ref, wq_hbm, wk_hbm, wv_hbm, wo_hbm, w1_hbm, b1_ref, w2_hbm, b2_ref,
            c_ref, wmod_hbm, out_hbm,
            wqkv, wo, w1, w2, xs, outs, ring, oring, x1buf, mod, stage, mstage, sems):
    NCH = 3 * (H // HC)
    w_src = (wq_hbm.bitcast(U32), wk_hbm.bitcast(U32), wv_hbm.bitcast(U32))

    def qkv_copy(c):
        m, g = divmod(c, H // HC)
        return pltpu.make_async_copy(w_src[m].at[:, pl.ds(g * (HC // 2), HC // 2), :],
                                     stage.at[c % 2], sems.at[c % 2])

    def mod_copy(j):
        return pltpu.make_async_copy(wmod_hbm.at[:, pl.ds(j * DM, DM)], mstage.at[j % 2],
                                     sems.at[2 + j % 2])

    x_copy0 = pltpu.make_async_copy(x_hbm.at[pl.ds(0, LEAD)], xs.at[pl.ds(0, LEAD)], sems.at[4])
    x_copy1 = pltpu.make_async_copy(x_hbm.at[pl.ds(LEAD, S - LEAD)], xs.at[pl.ds(LEAD, S - LEAD)],
                                    sems.at[5])
    wo_copy = pltpu.make_async_copy(wo_hbm.bitcast(U32), wo, sems.at[6])
    w1_copy = pltpu.make_async_copy(w1_hbm.bitcast(U32), w1, sems.at[7])
    w2_copy = pltpu.make_async_copy(w2_hbm.bitcast(U32), w2, sems.at[8])

    cv = c_ref[...].astype(F32)
    sc = jnp.broadcast_to(cv * jax.nn.sigmoid(cv), (16, DM)).astype(BF16)

    def mod_chunk(j):
        mod_copy(j).wait()
        mod[:, pl.ds(j * DM, DM)] = _dot(sc, mstage[j % 2])[:8]

    mod_copy(0).start()
    mod_copy(1).start()
    x_copy0.start()
    qkv_copy(0).start()
    qkv_copy(1).start()
    mod_chunk(0)
    mod_chunk(1)
    mod_copy(2).start()
    x_copy0.wait()

    sa, ca = mod[0:1, 0:DM], mod[0:1, DM:2 * DM]
    h0 = _ln_mod(xs[0:LEAD].astype(F32), ca, sa).astype(BF16)
    for c in range(NCH):
        qkv_copy(c).wait()
        st = stage.at[c % 2]
        for j in range(HC // 2):
            a = st[pl.ds(0, DM // 2, stride=2), j, :]
            b = st[pl.ds(1, DM // 2, stride=2), j, :]
            wqkv[c * HC + 2 * j] = (a & U32(0xFFFF)) | (b << 16)
            wqkv[c * HC + 2 * j + 1] = (a >> 16) | (b & U32(0xFFFF0000))
        if c + 2 < NCH:
            qkv_copy(c + 2).start()
        elif c + 2 == NCH:
            wo_copy.start()
        else:
            w1_copy.start()
            w2_copy.start()
            x_copy1.start()
        for t in range(c * HC, (c + 1) * HC):
            ring[t, pl.ds(ROFF, LEAD), :] = _dot(h0, _w(wqkv[t]))
    mod_chunk(2)
    mod_copy(3).start()
    mod_copy(4).start()
    mod_chunk(3)
    mod_copy(5).start()
    mod_chunk(4)
    mod_chunk(5)
    wo_copy.wait()
    w1_copy.wait()
    w2_copy.wait()
    x_copy1.wait()

    ga = mod[0:1, 2 * DM:3 * DM]
    sb, cb, gb = mod[0:1, 3 * DM:4 * DM], mod[0:1, 4 * DM:5 * DM], mod[0:1, 5 * DM:6 * DM]
    b1 = b1_ref[...].astype(F32)
    b2 = b2_ref[...].astype(F32)

    def ffn(x1):
        h2 = _ln_mod(x1, cb, sb).astype(BF16)
        u = _gelu(_dot(h2, _w(w1[...])) + b1).astype(BF16)
        return (x1 + gb * (_dot(u, _w(w2[...])) + b2)).astype(BF16)

    L = M + SEG
    row = lax.broadcasted_iota(jnp.int32, (L, L), 0)
    col = lax.broadcasted_iota(jnp.int32, (L, L), 1)
    mask = (row < M) | (row >= col)
    scale = float(DH) ** -0.5

    def step(s, mem, hx):
        lhs = jnp.concatenate([mem, hx], axis=0).astype(BF16)
        wslot = pl.multiple_of((LEAD + ROFF + TOK * s) % RING, 8)
        r0 = pl.multiple_of((SEG * s + ROFF) % RING, 16)
        r1 = pl.multiple_of((SEG * s + ROFF + 16) % RING, 16)
        oslot = pl.multiple_of((SEG * s) % RING, 32)
        mrow = []
        for t in range(3 * H):
            r = _dot(lhs, _w(wqkv[t]))
            ring[t, pl.ds(wslot, TOK), :] = r[M:]
            mrow.append(r[:M])

        def ext(t):
            return jnp.concatenate([mrow[t], ring[t, pl.ds(r0, 16), :], ring[t, pl.ds(r1, 16), :]],
                                   axis=0).astype(BF16)

        om = []
        for h in range(H):
            q, k, v = ext(h), ext(H + h), ext(2 * H + h)
            sc_ = lax.dot_general(q, k, (((1,), (1,)), ((), ())), preferred_element_type=F32) * scale
            sc_ = jnp.where(mask, sc_, -1e9)
            p = jnp.exp(sc_ - jnp.max(sc_, axis=-1, keepdims=True))
            p = p / jnp.sum(p, axis=-1, keepdims=True)
            o = _dot(p.astype(BF16), v)
            oring[pl.ds(oslot, SEG), pl.ds(h * DH, DH)] = o[M:]
            om.append(o[:M])
        rslot = pl.multiple_of((TOK * s) % RING, 8)
        lhs2 = jnp.concatenate([jnp.concatenate(om, axis=1), oring[pl.ds(rslot, TOK), :]], axis=0)
        r2 = _dot(lhs2.astype(BF16), _w(wo[...]))
        return r2[:M], r2[M:]

    x1buf[pl.ds(0, BLK), :] = jnp.zeros((BLK, DM), F32)

    def body(i, mem):
        hx = _ln_mod(xs[pl.ds(pl.multiple_of(LEAD + BLK * i, 16), BLK), :].astype(F32), ca, sa)
        prev = pl.multiple_of(jnp.maximum(BLK * (i - 1), 0), 16)
        outs[pl.ds(prev, BLK), :] = ffn(x1buf[pl.ds(0, BLK), :])
        mem, ya = step(2 * i, mem, hx[:TOK])
        mem, yb = step(2 * i + 1, mem, hx[TOK:])
        xr = xs[pl.ds(pl.multiple_of(BLK * i, 16), BLK), :].astype(F32)
        x1buf[pl.ds(0, BLK), :] = xr + ga * jnp.concatenate([ya, yb], axis=0)
        return mem

    lax.fori_loop(0, NIT, body, mem0_ref[...].astype(F32))

    DONE = BLK * (NIT - 1)
    out_copy0 = pltpu.make_async_copy(outs.at[pl.ds(0, DONE)], out_hbm.at[pl.ds(0, DONE)], sems.at[9])
    out_copy0.start()
    outs[pl.ds(DONE, BLK), :] = ffn(x1buf[pl.ds(0, BLK), :])
    EB = 256
    for e in range(LEAD // EB):
        p0 = NSEG * TOK + e * EB
        o = jnp.concatenate([oring[pl.ds((p0 + 64 * q) % RING, 64), :] for q in range(EB // 64)], axis=0)
        y = _dot(o.astype(BF16), _w(wo[...]))
        x1 = xs[pl.ds(p0, EB), :].astype(F32) + ga * y
        outs[pl.ds(p0, EB), :] = ffn(x1)
    out_copy1 = pltpu.make_async_copy(outs.at[pl.ds(DONE, S - DONE)], out_hbm.at[pl.ds(DONE, S - DONE)],
                                      sems.at[10])
    out_copy1.start()
    out_copy0.wait()
    out_copy1.wait()


@functools.partial(jax.jit, static_argnames=("A_seg_len",))
def pallas_adaLN_cond__memory_aug_recurrent_mem_tr__dense_activation_gelu__prompt_kernel(
    A_x, A_mem0, A_Wq, A_Wk, A_Wv, A_Wo, A_seg_len, B_x, B_w1, B_b1, B_w2, B_b2, c, w_mod,
):
    del B_x
    assert A_x.shape == (1, S, DM) and int(A_seg_len) == SEG
    hbm = pl.BlockSpec(memory_space=pl.ANY)
    vmem = pl.BlockSpec(memory_space=pltpu.VMEM)
    out = pl.pallas_call(
        _kernel,
        out_shape=jax.ShapeDtypeStruct((S, DM), BF16),
        in_specs=[hbm, vmem, hbm, hbm, hbm, hbm, hbm, vmem, hbm, vmem, vmem, hbm],
        out_specs=hbm,
        scratch_shapes=[
            pltpu.VMEM((3 * H, DM // 2, DH), U32),
            pltpu.VMEM((H * DH // 2, DM), U32),
            pltpu.VMEM((DM // 2, FF), U32),
            pltpu.VMEM((FF // 2, DM), U32),
            pltpu.VMEM((S, DM), BF16),
            pltpu.VMEM((S, DM), BF16),
            pltpu.VMEM((3 * H, RING, DH), F32),
            pltpu.VMEM((RING, H * DH), F32),
            pltpu.VMEM((BLK, DM), F32),
            pltpu.VMEM((8, 6 * DM), F32),
            pltpu.VMEM((2, DM, HC // 2, DH), U32),
            pltpu.VMEM((2, DM, DM), BF16),
            pltpu.SemaphoreType.DMA((11,)),
        ],
        compiler_params=pltpu.CompilerParams(vmem_limit_bytes=124 * 1024 * 1024),
    )(A_x.reshape(S, DM), A_mem0.reshape(M, DM), A_Wq, A_Wk, A_Wv, A_Wo.reshape(H * DH, DM),
      B_w1, B_b1.reshape(1, FF), B_w2, B_b2.reshape(1, DM), c, w_mod)
    return out.reshape(1, S, DM)
```

```python
import functools

import jax
import jax.numpy as jnp
import numpy as np
from jax import lax
import jax.experimental.pallas as pl
import jax.experimental.pallas.tpu as pltpu

S, DM, H, DH, M, SEG, FF = 2048, 1024, 32, 128, 8, 32, 3584
NSEG = S // SEG
TOK = 24
LEAD = S - NSEG * TOK
RING = 576
ROFF = (-LEAD) % TOK
NIT = NSEG // 2
BLK = 2 * TOK
HC = 16
EPS = 1e-5
F32, BF16, U32 = jnp.float32, jnp.bfloat16, jnp.uint32


def _ln_mod(x, scale, shift):
    m = jnp.mean(x, axis=-1, keepdims=True)
    xc = x - m
    v = jnp.mean(xc * xc, axis=-1, keepdims=True)
    return xc * lax.rsqrt(v + EPS) * (1.0 + scale) + shift


def _gelu(x):
    c = float(np.sqrt(2.0 / np.pi))
    return 0.5 * x * (1.0 + jnp.tanh(c * (x + 0.044715 * (x * x * x))))


def _w(ref_val):
    return pltpu.bitcast(ref_val, BF16)


def _dot(a, b):
    return jnp.dot(a, b, preferred_element_type=F32)


def _kernel(x_hbm, mem0_ref, wq_hbm, wk_hbm, wv_hbm, wo_hbm, w1_hbm, b1_ref, w2_hbm, b2_ref,
            c_ref, wmod_hbm, out_hbm,
            wqkv, wo, w1, w2, xs, outs, ring, oring, x1buf, hxbuf, ubuf, mod, stage, mstage, sems):
    NCH = 3 * (H // HC)
    w_src = (wq_hbm.bitcast(U32), wk_hbm.bitcast(U32), wv_hbm.bitcast(U32))

    def qkv_copy(c):
        m, g = divmod(c, H // HC)
        return pltpu.make_async_copy(w_src[m].at[:, pl.ds(g * (HC // 2), HC // 2), :],
                                     stage.at[c % 2], sems.at[c % 2])

    def mod_copy(j):
        return pltpu.make_async_copy(wmod_hbm.at[:, pl.ds(j * DM, DM)], mstage.at[j % 2],
                                     sems.at[2 + j % 2])

    x_copy0 = pltpu.make_async_copy(x_hbm.at[pl.ds(0, LEAD)], xs.at[pl.ds(0, LEAD)], sems.at[4])
    x_copy1 = pltpu.make_async_copy(x_hbm.at[pl.ds(LEAD, S - LEAD)], xs.at[pl.ds(LEAD, S - LEAD)],
                                    sems.at[5])
    wo_copy = pltpu.make_async_copy(wo_hbm.bitcast(U32), wo, sems.at[6])
    w1_copy = pltpu.make_async_copy(w1_hbm.bitcast(U32), w1, sems.at[7])
    w2_copy = pltpu.make_async_copy(w2_hbm.bitcast(U32), w2, sems.at[8])

    cv = c_ref[...].astype(F32)
    sc = jnp.broadcast_to(cv * jax.nn.sigmoid(cv), (16, DM)).astype(BF16)

    def mod_chunk(j):
        mod_copy(j).wait()
        mod[:, pl.ds(j * DM, DM)] = _dot(sc, mstage[j % 2])[:8]

    mod_copy(0).start()
    mod_copy(1).start()
    x_copy0.start()
    qkv_copy(0).start()
    qkv_copy(1).start()
    mod_chunk(0)
    mod_chunk(1)
    mod_copy(2).start()
    x_copy0.wait()

    sa, ca = mod[0:1, 0:DM], mod[0:1, DM:2 * DM]
    h0buf = outs.at[pl.ds(0, LEAD)]
    h0buf[...] = _ln_mod(xs[0:LEAD].astype(F32), ca, sa).astype(BF16)
    def relayout(c):
        qkv_copy(c).wait()
        st = stage.at[c % 2].reshape(DM * HC // 2, DH)
        for j in range(HC // 2):
            a = st[pl.ds(j, DM // 2, stride=HC), :]
            b = st[pl.ds(HC // 2 + j, DM // 2, stride=HC), :]
            wqkv[c * HC + 2 * j] = (a & U32(0xFFFF)) | (b << 16)
            wqkv[c * HC + 2 * j + 1] = (a >> 16) | (b & U32(0xFFFF0000))
        if c + 2 < NCH:
            qkv_copy(c + 2).start()

    relayout(0)
    for c in range(NCH):
        if c == 0:
            wo_copy.start()
        elif c == 2:
            mod_chunk(2)
            mod_copy(3).start()
            mod_copy(4).start()
        elif c == 3:
            x_copy1.start()
            w1_copy.start()
        elif c == 4:
            mod_chunk(3)
            mod_copy(5).start()
            mod_chunk(4)
            w2_copy.start()

        for t in range(c * HC, (c + 1) * HC):
            ring[t, pl.ds(ROFF, LEAD), :] = _dot(h0buf[...], _w(wqkv[t]))
            if t == c * HC + HC // 2 and c + 1 < NCH:
                relayout(c + 1)
    mod_chunk(5)
    wo_copy.wait()
    x_copy1.wait()

    ga = mod[0:1, 2 * DM:3 * DM]
    sb, cb, gb = mod[0:1, 3 * DM:4 * DM], mod[0:1, 4 * DM:5 * DM], mod[0:1, 5 * DM:6 * DM]
    b1 = b1_ref[...].astype(F32)
    b2 = b2_ref[...].astype(F32)

    def ffn(x1):
        h2 = _ln_mod(x1, cb, sb).astype(BF16)
        u = _gelu(_dot(h2, _w(w1[...])) + b1).astype(BF16)
        return (x1 + gb * (_dot(u, _w(w2[...])) + b2)).astype(BF16)

    L = M + SEG
    row = lax.broadcasted_iota(jnp.int32, (L, DH), 0)
    col = lax.broadcasted_iota(jnp.int32, (L, DH), 1)
    mask = (col < L) & ((row < M) | (row >= col))
    zpad = jnp.zeros((DH - L, DH), F32)
    scale = float(DH) ** -0.5

    def step(s, mem, hx, fill):
        lhs = jnp.concatenate([mem, hx], axis=0).astype(BF16)
        wslot = pl.multiple_of((LEAD + ROFF + TOK * s) % RING, 8)
        r0 = pl.multiple_of((SEG * s + ROFF) % RING, 16)
        r1 = pl.multiple_of((SEG * s + ROFF + 16) % RING, 16)
        oslot = pl.multiple_of((SEG * s) % RING, 32)
        mrow = []
        for t in range(3 * H):
            r = _dot(lhs, _w(wqkv[t]))
            ring[t, pl.ds(wslot, TOK), :] = r[M:]
            mrow.append(r[:M])

        def ext(t, pad):
            parts = [mrow[t], ring[t, pl.ds(r0, 16), :], ring[t, pl.ds(r1, 16), :]]
            return jnp.concatenate(parts + [zpad] * pad, axis=0)

        om = []
        G = 8
        for h0 in range(0, H, G):
            hs = range(h0, h0 + G)
            ss = []
            for h in hs:
                q = (ext(h, 0) * scale).astype(BF16)
                k = ext(H + h, 1).astype(BF16)
                ss.append(lax.dot_general(q, k, (((1,), (1,)), ((), ())), preferred_element_type=F32))
            ps = []
            for sc_ in ss:
                sc_ = jnp.where(mask, sc_, -1e9)
                p = jnp.exp(sc_ - jnp.max(sc_, axis=-1, keepdims=True))
                l = jnp.sum(p, axis=-1, keepdims=True)
                r = pl.reciprocal(l, approx=True)
                r = r * (2.0 - l * r)
                ps.append((p * r).astype(BF16))
                if fill:
                    fill.pop(0)()
            for h, p in zip(hs, ps):
                o = _dot(p, ext(2 * H + h, 1).astype(BF16))
                oring[pl.ds(oslot, SEG), pl.ds(h * DH, DH)] = o[M:]
                om.append(o[:M])
        rslot = pl.multiple_of((TOK * s) % RING, 8)
        lhs2 = jnp.concatenate([jnp.concatenate(om, axis=1), oring[pl.ds(rslot, TOK), :]], axis=0)
        r2 = _dot(lhs2.astype(BF16), _w(wo[...]))
        return r2[:M], r2[M:]

    def ln_block(i):
        r = pl.multiple_of(jnp.minimum(LEAD + BLK * i, S - BLK), 16)
        hxbuf[...] = _ln_mod(xs[pl.ds(r, BLK), :].astype(F32), ca, sa)

    x1buf[...] = jnp.zeros((BLK, DM), F32)
    ln_block(0)
    NU, KP = FF // 128, 4
    KC = FF // KP

    def body(i, mem, ffn_on=True):
        x1 = x1buf[...]
        h2 = _ln_mod(x1, cb, sb).astype(BF16)
        prev = pl.multiple_of(jnp.maximum(BLK * (i - 1), 0), 16)
        acc = {}

        def up(n):
            cs = pl.ds(n * 128, 128)
            ubuf[:, cs] = _gelu(_dot(h2, _w(w1[:, cs])) + b1[:, n * 128:(n + 1) * 128]).astype(BF16)

        def down(n, k):
            cs = pl.ds(n * 128, 128)
            d = _dot(ubuf[:, pl.ds(k * KC, KC)], _w(w2[pl.ds(k * KC // 2, KC // 2), cs]))
            acc[n] = d if k == 0 else acc[n] + d
            if k == KP - 1:
                sl = slice(n * 128, (n + 1) * 128)
                outs[pl.ds(prev, BLK), cs] = (x1[:, sl] + gb[:, sl] * (acc[n] + b2[:, sl])).astype(BF16)

        ups = [functools.partial(up, n) for n in range(NU)]
        downs = [functools.partial(down, n, k) for n in range(DM // 128) for k in range(KP)]
        if not ffn_on:
            ups, downs = [], []
        mem, ya = step(2 * i, mem, hxbuf[0:TOK, :], ups)
        for f in downs[:24]:
            f()
        mem, yb = step(2 * i + 1, mem, hxbuf[TOK:BLK, :], [])
        for f in downs[24:]:
            f()
        ln_block(i + 1)
        xr = xs[pl.ds(pl.multiple_of(BLK * i, 16), BLK), :].astype(F32)
        x1buf[...] = xr + ga * jnp.concatenate([ya, yb], axis=0)
        return mem

    mem1 = body(0, mem0_ref[...].astype(F32), ffn_on=False)
    w1_copy.wait()
    w2_copy.wait()
    lax.fori_loop(1, NIT, body, mem1)

    DONE = BLK * (NIT - 1)
    out_copy0 = pltpu.make_async_copy(outs.at[pl.ds(0, DONE)], out_hbm.at[pl.ds(0, DONE)], sems.at[9])
    out_copy0.start()
    outs[pl.ds(DONE, BLK), :] = ffn(x1buf[...])
    EB = 256

    def tail(e, carry):
        p0 = pl.multiple_of(NSEG * TOK + e * EB, EB)
        o = jnp.concatenate([oring[pl.ds(pl.multiple_of((p0 + 64 * q) % RING, 64), 64), :]
                             for q in range(EB // 64)], axis=0)
        y = _dot(o.astype(BF16), _w(wo[...]))
        x1 = xs[pl.ds(p0, EB), :].astype(F32) + ga * y
        outs[pl.ds(p0, EB), :] = ffn(x1)
        return carry

    lax.fori_loop(0, LEAD // EB, tail, 0)
    out_copy1 = pltpu.make_async_copy(outs.at[pl.ds(DONE, S - DONE)], out_hbm.at[pl.ds(DONE, S - DONE)],
                                      sems.at[10])
    out_copy1.start()
    out_copy0.wait()
    out_copy1.wait()


@functools.partial(jax.jit, static_argnames=("A_seg_len",))
def pallas_adaLN_cond__memory_aug_recurrent_mem_tr__dense_activation_gelu__prompt_kernel(
    A_x, A_mem0, A_Wq, A_Wk, A_Wv, A_Wo, A_seg_len, B_x, B_w1, B_b1, B_w2, B_b2, c, w_mod,
):
    del B_x
    assert A_x.shape == (1, S, DM) and int(A_seg_len) == SEG
    hbm = pl.BlockSpec(memory_space=pl.ANY)
    vmem = pl.BlockSpec(memory_space=pltpu.VMEM)
    out = pl.pallas_call(
        _kernel,
        out_shape=jax.ShapeDtypeStruct((S, DM), BF16),
        in_specs=[hbm, vmem, hbm, hbm, hbm, hbm, hbm, vmem, hbm, vmem, vmem, hbm],
        out_specs=hbm,
        scratch_shapes=[
            pltpu.VMEM((3 * H, DM // 2, DH), U32),
            pltpu.VMEM((H * DH // 2, DM), U32),
            pltpu.VMEM((DM // 2, FF), U32),
            pltpu.VMEM((FF // 2, DM), U32),
            pltpu.VMEM((S, DM), BF16),
            pltpu.VMEM((S, DM), BF16),
            pltpu.VMEM((3 * H, RING, DH), F32),
            pltpu.VMEM((RING, H * DH), F32),
            pltpu.VMEM((BLK, DM), F32),
            pltpu.VMEM((BLK, DM), F32),
            pltpu.VMEM((BLK, FF), BF16),
            pltpu.VMEM((8, 6 * DM), F32),
            pltpu.VMEM((2, DM, HC // 2, DH), U32),
            pltpu.VMEM((2, DM, DM), BF16),
            pltpu.SemaphoreType.DMA((11,)),
        ],
        compiler_params=pltpu.CompilerParams(vmem_limit_bytes=124 * 1024 * 1024),
    )(A_x.reshape(S, DM), A_mem0.reshape(M, DM), A_Wq, A_Wk, A_Wv, A_Wo.reshape(H * DH, DM),
      B_w1, B_b1.reshape(1, FF), B_w2, B_b2.reshape(1, DM), c, w_mod)
    return out.reshape(1, S, DM)
```

```python
import functools

import jax
import jax.numpy as jnp
import numpy as np
from jax import lax
import jax.experimental.pallas as pl
import jax.experimental.pallas.tpu as pltpu

S, DM, H, DH, M, SEG, FF = 2048, 1024, 32, 128, 8, 32, 3584
NSEG = S // SEG
TOK = 24
TAILN = S - NSEG * TOK
LEAD = TAILN + 32
RING = 576
ROFF = (-LEAD) % TOK
NIT = NSEG // 2
BLK = 2 * TOK
HC = 16
EPS = 1e-5
F32, BF16, U32 = jnp.float32, jnp.bfloat16, jnp.uint32


def _ln_mod(x, scale, shift):
    m = jnp.mean(x, axis=-1, keepdims=True)
    xc = x - m
    v = jnp.mean(xc * xc, axis=-1, keepdims=True)
    return xc * lax.rsqrt(v + EPS) * (1.0 + scale) + shift


def _gelu(x):
    c = float(np.sqrt(2.0 / np.pi))
    return 0.5 * x * (1.0 + jnp.tanh(c * (x + 0.044715 * (x * x * x))))


def _w(ref_val):
    return pltpu.bitcast(ref_val, BF16)


def _dot(a, b):
    return jnp.dot(a, b, preferred_element_type=F32)


def _kernel(x_hbm, mem0_ref, wq_hbm, wk_hbm, wv_hbm, wo_hbm, w1_hbm, b1_ref, w2_hbm, b2_ref,
            c_ref, wmod_hbm, out_hbm,
            wqkv, wo, w1, w2, xs, outs, ring, oring, x1buf, hxbuf, ubuf, mod, stage, mstage, sems):
    NCH = 3 * (H // HC)
    w_src = (wq_hbm.bitcast(U32), wk_hbm.bitcast(U32), wv_hbm.bitcast(U32))

    def qkv_copy(c):
        m, g = divmod(c, H // HC)
        return pltpu.make_async_copy(w_src[m].at[:, pl.ds(g * (HC // 2), HC // 2), :],
                                     stage.at[c % 2], sems.at[c % 2])

    def mod_copy(j):
        return pltpu.make_async_copy(wmod_hbm.at[:, pl.ds(j * DM, DM)], mstage.at[j % 2],
                                     sems.at[2 + j % 2])

    x_copy0 = pltpu.make_async_copy(x_hbm.at[pl.ds(0, LEAD)], xs.at[pl.ds(0, LEAD)], sems.at[4])
    x_copy1 = pltpu.make_async_copy(x_hbm.at[pl.ds(LEAD, S - LEAD)], xs.at[pl.ds(LEAD, S - LEAD)],
                                    sems.at[5])
    wo_copy = pltpu.make_async_copy(wo_hbm.bitcast(U32), wo, sems.at[6])
    w1_copy = pltpu.make_async_copy(w1_hbm.bitcast(U32), w1, sems.at[7])
    w2_copy = pltpu.make_async_copy(w2_hbm.bitcast(U32), w2, sems.at[8])

    cv = c_ref[...].astype(F32)
    sc = jnp.broadcast_to(cv * jax.nn.sigmoid(cv), (16, DM)).astype(BF16)

    def mod_chunk(j):
        mod_copy(j).wait()
        mod[:, pl.ds(j * DM, DM)] = _dot(sc, mstage[j % 2])[:8]

    xs[pl.ds(S, 32), :] = jnp.zeros((32, DM), BF16)
    mod_copy(0).start()
    mod_copy(1).start()
    x_copy0.start()
    qkv_copy(0).start()
    qkv_copy(1).start()
    mod_chunk(0)
    mod_chunk(1)
    mod_copy(2).start()
    x_copy0.wait()

    sa, ca = mod[0:1, 0:DM], mod[0:1, DM:2 * DM]
    h0buf = outs.at[pl.ds(0, LEAD)]
    h0buf[...] = _ln_mod(xs[0:LEAD].astype(F32), ca, sa).astype(BF16)
    def relayout(c):
        qkv_copy(c).wait()
        st = stage.at[c % 2].reshape(DM * HC // 2, DH)
        for j in range(HC // 2):
            a = st[pl.ds(j, DM // 2, stride=HC), :]
            b = st[pl.ds(HC // 2 + j, DM // 2, stride=HC), :]
            wqkv[c * HC + 2 * j] = (a & U32(0xFFFF)) | (b << 16)
            wqkv[c * HC + 2 * j + 1] = (a >> 16) | (b & U32(0xFFFF0000))
        if c + 2 < NCH:
            qkv_copy(c + 2).start()

    relayout(0)
    for c in range(NCH):
        if c == 0:
            wo_copy.start()
        elif c == 2:
            mod_chunk(2)
            mod_copy(3).start()
            mod_copy(4).start()
        elif c == 3:
            x_copy1.start()
            w1_copy.start()
        elif c == 4:
            mod_chunk(3)
            mod_copy(5).start()
            mod_chunk(4)
            w2_copy.start()

        for t in range(c * HC, (c + 1) * HC):
            ring[t, pl.ds(ROFF, LEAD), :] = _dot(h0buf[...], _w(wqkv[t]))
            if t == c * HC + HC // 2 and c + 1 < NCH:
                relayout(c + 1)
    mod_chunk(5)
    wo_copy.wait()
    x_copy1.wait()

    ga = mod[0:1, 2 * DM:3 * DM]
    sb, cb, gb = mod[0:1, 3 * DM:4 * DM], mod[0:1, 4 * DM:5 * DM], mod[0:1, 5 * DM:6 * DM]
    b1 = b1_ref[...].astype(F32)
    b2 = b2_ref[...].astype(F32)

    def ffn(x1):
        h2 = _ln_mod(x1, cb, sb).astype(BF16)
        u = _gelu(_dot(h2, _w(w1[...])) + b1).astype(BF16)
        return (x1 + gb * (_dot(u, _w(w2[...])) + b2)).astype(BF16)

    L = M + SEG
    row = lax.broadcasted_iota(jnp.int32, (L, DH), 0)
    col = lax.broadcasted_iota(jnp.int32, (L, DH), 1)
    mask = (col < L) & ((row < M) | (row >= col))
    zpad = jnp.zeros((DH - L, DH), F32)
    scale = float(DH) ** -0.5

    G = 8

    def step(s, mem, hx, fill):
        lhs = jnp.concatenate([mem, hx], axis=0).astype(BF16)
        wslot = pl.multiple_of((LEAD + ROFF + TOK * s) % RING, 8)
        rs = [pl.multiple_of((SEG * s + ROFF + 8 * q) % RING, 8) for q in range(4)]
        oslot = pl.multiple_of((SEG * s) % RING, 32)
        rslot = pl.multiple_of((TOK * s) % RING, 8)
        mrow, lhs2, acc, tokr = {}, {}, {}, {}

        def proj(t):
            r = _dot(lhs, _w(wqkv[t]))
            tokr[t] = r[M:]
            mrow[t] = r[:M]

        def ext(t, pad):
            parts = [mrow[t]] + [ring[t, pl.ds(r, 8), :] for r in rs]
            return jnp.concatenate(parts + [zpad] * pad, axis=0)

        def attend(h):
            q = (ext(h, 0) * scale).astype(BF16)
            k = ext(H + h, 1).astype(BF16)
            sc_ = lax.dot_general(q, k, (((1,), (1,)), ((), ())), preferred_element_type=F32)
            sc_ = jnp.where(mask, sc_, -1e9)
            p = jnp.exp(sc_ - jnp.max(sc_, axis=-1, keepdims=True))
            l = jnp.sum(p, axis=-1, keepdims=True)
            r = pl.reciprocal(l, approx=True)
            r = r * (2.0 - l * r)
            o = _dot((p * r).astype(BF16), ext(2 * H + h, 1).astype(BF16))
            cs = pl.ds(h * DH, DH)
            oring[pl.ds(oslot, SEG), cs] = o[M:]
            lhs2[h] = jnp.concatenate([o[:M], oring[pl.ds(rslot, TOK), cs]], axis=0).astype(BF16)

        def outp(g, n):
            a = jnp.concatenate([lhs2[h] for h in range(g * G, (g + 1) * G)], axis=1)
            d = _dot(a, _w(wo[pl.ds(g * G * DH // 2, G * DH // 2), pl.ds(n * 128, 128)]))
            acc[n] = d if g == 0 else acc[n] + d

        NG = H // G
        for g in range(NG + 2):
            for j in range(G):
                if g < NG:
                    for m in range(3):
                        proj(m * H + g * G + j)
                if 1 <= g <= NG:
                    attend((g - 1) * G + j)
                if g >= 2:
                    outp(g - 2, j)
                if g >= NG:
                    for _ in range(2):
                        if fill:
                            fill.pop(0)()
        for t in range(3 * H):
            ring[t, pl.ds(wslot, TOK), :] = tokr[t]
        r2 = jnp.concatenate([acc[n] for n in range(DM // 128)], axis=1)
        return r2[:M], r2[M:]

    def ln_block(i):
        r = pl.multiple_of(jnp.minimum(LEAD + BLK * i, S + 32 - BLK), 16)
        hxbuf[...] = _ln_mod(xs[pl.ds(r, BLK), :].astype(F32), ca, sa)

    x1buf[...] = jnp.zeros((BLK, DM), F32)
    ln_block(0)
    NU, KP = FF // 128, 4
    KC = FF // KP

    def body(i, mem, ffn_on=True):
        x1 = x1buf[...]
        h2 = _ln_mod(x1, cb, sb).astype(BF16)
        prev = pl.multiple_of(jnp.maximum(BLK * (i - 1), 0), 16)
        acc = {}

        def up(n):
            cs = pl.ds(n * 128, 128)
            ubuf[:, cs] = _gelu(_dot(h2, _w(w1[:, cs])) + b1[:, n * 128:(n + 1) * 128]).astype(BF16)

        def down(n, k):
            cs = pl.ds(n * 128, 128)
            d = _dot(ubuf[:, pl.ds(k * KC, KC)], _w(w2[pl.ds(k * KC // 2, KC // 2), cs]))
            acc[n] = d if k == 0 else acc[n] + d
            if k == KP - 1:
                sl = slice(n * 128, (n + 1) * 128)
                outs[pl.ds(prev, BLK), cs] = (x1[:, sl] + gb[:, sl] * (acc[n] + b2[:, sl])).astype(BF16)

        ups = [functools.partial(up, n) for n in range(NU)]
        downs = [functools.partial(down, n, k) for n in range(DM // 128) for k in range(KP)]
        if not ffn_on:
            ups, downs = [], []
        mem, ya = step(2 * i, mem, hxbuf[0:TOK, :], ups)
        for f in downs[:24]:
            f()
        mem, yb = step(2 * i + 1, mem, hxbuf[TOK:BLK, :], [])
        for f in downs[24:]:
            f()
        ln_block(i + 1)
        xr = xs[pl.ds(pl.multiple_of(BLK * i, 16), BLK), :].astype(F32)
        x1buf[...] = xr + ga * jnp.concatenate([ya, yb], axis=0)
        return mem

    mem1 = body(0, mem0_ref[...].astype(F32), ffn_on=False)
    w1_copy.wait()
    w2_copy.wait()
    lax.fori_loop(1, NIT, body, mem1)

    DONE = BLK * (NIT - 1)
    out_copy0 = pltpu.make_async_copy(outs.at[pl.ds(0, DONE)], out_hbm.at[pl.ds(0, DONE)], sems.at[9])
    out_copy0.start()
    outs[pl.ds(DONE, BLK), :] = ffn(x1buf[...])
    EB = 256

    def tail(e, carry):
        p0 = pl.multiple_of(NSEG * TOK + e * EB, EB)
        o = jnp.concatenate([oring[pl.ds(pl.multiple_of((p0 + 64 * q) % RING, 64), 64), :]
                             for q in range(EB // 64)], axis=0)
        y = _dot(o.astype(BF16), _w(wo[...]))
        x1 = xs[pl.ds(p0, EB), :].astype(F32) + ga * y
        outs[pl.ds(p0, EB), :] = ffn(x1)
        return carry

    lax.fori_loop(0, TAILN // EB, tail, 0)
    out_copy1 = pltpu.make_async_copy(outs.at[pl.ds(DONE, S - DONE)], out_hbm.at[pl.ds(DONE, S - DONE)],
                                      sems.at[10])
    out_copy1.start()
    out_copy0.wait()
    out_copy1.wait()


@functools.partial(jax.jit, static_argnames=("A_seg_len",))
def pallas_adaLN_cond__memory_aug_recurrent_mem_tr__dense_activation_gelu__prompt_kernel(
    A_x, A_mem0, A_Wq, A_Wk, A_Wv, A_Wo, A_seg_len, B_x, B_w1, B_b1, B_w2, B_b2, c, w_mod,
):
    del B_x
    assert A_x.shape == (1, S, DM) and int(A_seg_len) == SEG
    hbm = pl.BlockSpec(memory_space=pl.ANY)
    vmem = pl.BlockSpec(memory_space=pltpu.VMEM)
    out = pl.pallas_call(
        _kernel,
        out_shape=jax.ShapeDtypeStruct((S, DM), BF16),
        in_specs=[hbm, vmem, hbm, hbm, hbm, hbm, hbm, vmem, hbm, vmem, vmem, hbm],
        out_specs=hbm,
        scratch_shapes=[
            pltpu.VMEM((3 * H, DM // 2, DH), U32),
            pltpu.VMEM((H * DH // 2, DM), U32),
            pltpu.VMEM((DM // 2, FF), U32),
            pltpu.VMEM((FF // 2, DM), U32),
            pltpu.VMEM((S + 32, DM), BF16),
            pltpu.VMEM((S, DM), BF16),
            pltpu.VMEM((3 * H, RING, DH), F32),
            pltpu.VMEM((RING, H * DH), F32),
            pltpu.VMEM((BLK, DM), F32),
            pltpu.VMEM((BLK, DM), F32),
            pltpu.VMEM((BLK, FF), BF16),
            pltpu.VMEM((8, 6 * DM), F32),
            pltpu.VMEM((2, DM, HC // 2, DH), U32),
            pltpu.VMEM((2, DM, DM), BF16),
            pltpu.SemaphoreType.DMA((11,)),
        ],
        compiler_params=pltpu.CompilerParams(vmem_limit_bytes=124 * 1024 * 1024),
    )(A_x.reshape(S, DM), A_mem0.reshape(M, DM), A_Wq, A_Wk, A_Wv, A_Wo.reshape(H * DH, DM),
      B_w1, B_b1.reshape(1, FF), B_w2, B_b2.reshape(1, DM), c, w_mod)
    return out.reshape(1, S, DM)
```

```python
import functools

import jax
import jax.numpy as jnp
import numpy as np
from jax import lax
import jax.experimental.pallas as pl
import jax.experimental.pallas.tpu as pltpu

S, DM, H, DH, M, SEG, FF = 2048, 1024, 32, 128, 8, 32, 3584
NSEG = S // SEG
TOK = 24
TAILN = S - NSEG * TOK
LEAD = TAILN + 32
RING = 576
ROFF = (-LEAD) % TOK
NIT = NSEG // 2
BLK = 2 * TOK
HC = 16
EPS = 1e-5
F32, BF16, U32 = jnp.float32, jnp.bfloat16, jnp.uint32


def _ln_mod(x, scale, shift):
    m = jnp.mean(x, axis=-1, keepdims=True)
    xc = x - m
    v = jnp.mean(xc * xc, axis=-1, keepdims=True)
    return xc * lax.rsqrt(v + EPS) * (1.0 + scale) + shift


def _gelu(x):
    c = float(np.sqrt(2.0 / np.pi))
    return 0.5 * x * (1.0 + jnp.tanh(c * (x + 0.044715 * (x * x * x))))


def _w(ref_val):
    return pltpu.bitcast(ref_val, BF16)


def _dot(a, b):
    return jnp.dot(a, b, preferred_element_type=F32)


def _kernel(x_hbm, mem0_ref, wq_hbm, wk_hbm, wv_hbm, wo_hbm, w1_hbm, b1_ref, w2_hbm, b2_ref,
            c_ref, wmod_hbm, out_hbm,
            wqkv, wo, w1, w2, xs, outs, ring, oring, x1buf, hxbuf, ubuf, mod, stage, mstage, sems):
    NCH = 3 * (H // HC)
    w_src = (wq_hbm.bitcast(U32), wk_hbm.bitcast(U32), wv_hbm.bitcast(U32))

    def qkv_copy(c):
        m, g = divmod(c, H // HC)
        return pltpu.make_async_copy(w_src[m].at[:, pl.ds(g * (HC // 2), HC // 2), :],
                                     stage.at[c % 2], sems.at[c % 2])

    def mod_copy(j):
        return pltpu.make_async_copy(wmod_hbm.at[:, pl.ds(j * DM, DM)], mstage.at[j % 2],
                                     sems.at[2 + j % 2])

    x_copy0 = pltpu.make_async_copy(x_hbm.at[pl.ds(0, LEAD)], xs.at[pl.ds(0, LEAD)], sems.at[4])
    x_copy1 = pltpu.make_async_copy(x_hbm.at[pl.ds(LEAD, S - LEAD)], xs.at[pl.ds(LEAD, S - LEAD)],
                                    sems.at[5])
    wo_copy = pltpu.make_async_copy(wo_hbm.bitcast(U32), wo, sems.at[6])
    w1_copy = pltpu.make_async_copy(w1_hbm.bitcast(U32), w1, sems.at[7])
    w2_copy = pltpu.make_async_copy(w2_hbm.bitcast(U32), w2, sems.at[8])

    cv = c_ref[...].astype(F32)
    sc = jnp.broadcast_to(cv * jax.nn.sigmoid(cv), (16, DM)).astype(BF16)

    def mod_chunk(j):
        mod_copy(j).wait()
        mod[:, pl.ds(j * DM, DM)] = _dot(sc, mstage[j % 2])[:8]

    xs[pl.ds(S, 32), :] = jnp.zeros((32, DM), BF16)
    mod_copy(0).start()
    mod_copy(1).start()
    x_copy0.start()
    qkv_copy(0).start()
    mod_chunk(0)
    mod_chunk(1)
    qkv_copy(1).start()
    x_copy0.wait()
    mod_copy(2).start()

    sa, ca = mod[0:1, 0:DM], mod[0:1, DM:2 * DM]
    h0buf = outs.at[pl.ds(0, LEAD)]
    h0buf[...] = _ln_mod(xs[0:LEAD].astype(F32), ca, sa).astype(BF16)
    def relayout(c):
        qkv_copy(c).wait()
        st = stage.at[c % 2].reshape(DM * HC // 2, DH)
        for j in range(HC // 2):
            a = st[pl.ds(j, DM // 2, stride=HC), :]
            b = st[pl.ds(HC // 2 + j, DM // 2, stride=HC), :]
            wqkv[c * HC + 2 * j] = (a & U32(0xFFFF)) | (b << 16)
            wqkv[c * HC + 2 * j + 1] = (a >> 16) | (b & U32(0xFFFF0000))
        if c + 2 < NCH:
            qkv_copy(c + 2).start()

    relayout(0)
    for c in range(NCH):
        if c == 0:
            wo_copy.start()
        elif c == 2:
            mod_chunk(2)
            mod_copy(3).start()
            mod_copy(4).start()
        elif c == 3:
            x_copy1.start()
            w1_copy.start()
        elif c == 4:
            mod_chunk(3)
            mod_copy(5).start()
            mod_chunk(4)
            w2_copy.start()

        for t in range(c * HC, (c + 1) * HC):
            ring[t, pl.ds(ROFF, LEAD), :] = _dot(h0buf[...], _w(wqkv[t]))
            if t == c * HC + HC // 2 and c + 1 < NCH:
                relayout(c + 1)
    mod_chunk(5)
    wo_copy.wait()
    x_copy1.wait()

    ga = mod[0:1, 2 * DM:3 * DM]
    sb, cb, gb = mod[0:1, 3 * DM:4 * DM], mod[0:1, 4 * DM:5 * DM], mod[0:1, 5 * DM:6 * DM]
    b1 = b1_ref[...].astype(F32)
    b2 = b2_ref[...].astype(F32)

    def ffn(x1):
        h2 = _ln_mod(x1, cb, sb).astype(BF16)
        u = _gelu(_dot(h2, _w(w1[...])) + b1).astype(BF16)
        return (x1 + gb * (_dot(u, _w(w2[...])) + b2)).astype(BF16)

    L = M + SEG
    row = lax.broadcasted_iota(jnp.int32, (L, DH), 0)
    col = lax.broadcasted_iota(jnp.int32, (L, DH), 1)
    mask = (col < L) & ((row < M) | (row >= col))
    zpad = jnp.zeros((DH - L, DH), F32)
    scale = float(DH) ** -0.5

    G = 8

    def step(s, mem, hx, fill):
        lhs = jnp.concatenate([mem, hx], axis=0).astype(BF16)
        wslot = pl.multiple_of((LEAD + ROFF + TOK * s) % RING, 8)
        rs = [pl.multiple_of((SEG * s + ROFF + 8 * q) % RING, 8) for q in range(4)]
        oslot = pl.multiple_of((SEG * s) % RING, 32)
        rslot = pl.multiple_of((TOK * s) % RING, 8)
        mrow, lhs2, acc, tokr = {}, {}, {}, {}

        def proj(t):
            r = _dot(lhs, _w(wqkv[t]))
            tokr[t] = r[M:]
            mrow[t] = r[:M]

        def ext(t, pad):
            parts = [mrow[t]] + [ring[t, pl.ds(r, 8), :] for r in rs]
            return jnp.concatenate(parts + [zpad] * pad, axis=0)

        def attend(h):
            q = (ext(h, 0) * scale).astype(BF16)
            k = ext(H + h, 1).astype(BF16)
            sc_ = lax.dot_general(q, k, (((1,), (1,)), ((), ())), preferred_element_type=F32)
            sc_ = jnp.where(mask, sc_, -1e9)
            p = jnp.exp(sc_ - jnp.max(sc_, axis=-1, keepdims=True))
            l = jnp.sum(p, axis=-1, keepdims=True)
            r = pl.reciprocal(l, approx=True)
            r = r * (2.0 - l * r)
            o = _dot((p * r).astype(BF16), ext(2 * H + h, 1).astype(BF16))
            cs = pl.ds(h * DH, DH)
            oring[pl.ds(oslot, SEG), cs] = o[M:]
            lhs2[h] = jnp.concatenate([o[:M], oring[pl.ds(rslot, TOK), cs]], axis=0).astype(BF16)

        def outp(g, n):
            a = jnp.concatenate([lhs2[h] for h in range(g * G, (g + 1) * G)], axis=1)
            d = _dot(a, _w(wo[pl.ds(g * G * DH // 2, G * DH // 2), pl.ds(n * 128, 128)]))
            acc[n] = d if g == 0 else acc[n] + d

        NG = H // G
        for g in range(NG + 2):
            for j in range(G):
                if g < NG:
                    for m in range(3):
                        proj(m * H + g * G + j)
                if 1 <= g <= NG:
                    attend((g - 1) * G + j)
                if g >= 2:
                    outp(g - 2, j)
                if g >= NG:
                    for _ in range(2):
                        if fill:
                            fill.pop(0)()
        for t in range(3 * H):
            ring[t, pl.ds(wslot, TOK), :] = tokr[t]
        r2 = jnp.concatenate([acc[n] for n in range(DM // 128)], axis=1)
        return r2[:M], r2[M:]

    def ln_block(i):
        r = pl.multiple_of(jnp.minimum(LEAD + BLK * i, S + 32 - BLK), 16)
        hxbuf[...] = _ln_mod(xs[pl.ds(r, BLK), :].astype(F32), ca, sa)

    x1buf[...] = jnp.zeros((BLK, DM), F32)
    ln_block(0)
    NU, KP = FF // 128, 4
    KC = FF // KP

    def body(i, mem, ffn_on=True):
        x1 = x1buf[...]
        h2 = _ln_mod(x1, cb, sb).astype(BF16)
        prev = pl.multiple_of(jnp.maximum(BLK * (i - 1), 0), 16)
        acc = {}

        def up(n):
            cs = pl.ds(n * 128, 128)
            ubuf[:, cs] = _gelu(_dot(h2, _w(w1[:, cs])) + b1[:, n * 128:(n + 1) * 128]).astype(BF16)

        def down(n, k):
            cs = pl.ds(n * 128, 128)
            d = _dot(ubuf[:, pl.ds(k * KC, KC)], _w(w2[pl.ds(k * KC // 2, KC // 2), cs]))
            acc[n] = d if k == 0 else acc[n] + d
            if k == KP - 1:
                sl = slice(n * 128, (n + 1) * 128)
                outs[pl.ds(prev, BLK), cs] = (x1[:, sl] + gb[:, sl] * (acc[n] + b2[:, sl])).astype(BF16)

        ups = [functools.partial(up, n) for n in range(NU)]
        downs = [functools.partial(down, n, k) for n in range(DM // 128) for k in range(KP)]
        if not ffn_on:
            ups, downs = [], []
        mem, ya = step(2 * i, mem, hxbuf[0:TOK, :], ups)
        for f in downs[:24]:
            f()
        mem, yb = step(2 * i + 1, mem, hxbuf[TOK:BLK, :], [])
        for f in downs[24:]:
            f()
        ln_block(i + 1)
        xr = xs[pl.ds(pl.multiple_of(BLK * i, 16), BLK), :].astype(F32)
        x1buf[...] = xr + ga * jnp.concatenate([ya, yb], axis=0)
        return mem

    mem1 = body(0, mem0_ref[...].astype(F32), ffn_on=False)
    w1_copy.wait()
    w2_copy.wait()
    lax.fori_loop(1, NIT, body, mem1)

    DONE = BLK * (NIT - 1)
    out_copy0 = pltpu.make_async_copy(outs.at[pl.ds(0, DONE)], out_hbm.at[pl.ds(0, DONE)], sems.at[9])
    out_copy0.start()
    outs[pl.ds(DONE, BLK), :] = ffn(x1buf[...])
    EB = 256

    def tail(e, carry):
        p0 = NSEG * TOK + e * EB
        o = jnp.concatenate([oring[pl.ds((p0 + 64 * q) % RING, 64), :]
                             for q in range(EB // 64)], axis=0)
        y = _dot(o.astype(BF16), _w(wo[...]))
        x1 = xs[pl.ds(p0, EB), :].astype(F32) + ga * y
        outs[pl.ds(p0, EB), :] = ffn(x1)
        return carry

    for e in range(TAILN // EB):
        tail(e, 0)
    out_copy1 = pltpu.make_async_copy(outs.at[pl.ds(DONE, S - DONE)], out_hbm.at[pl.ds(DONE, S - DONE)],
                                      sems.at[10])
    out_copy1.start()
    out_copy0.wait()
    out_copy1.wait()


@functools.partial(jax.jit, static_argnames=("A_seg_len",))
def pallas_adaLN_cond__memory_aug_recurrent_mem_tr__dense_activation_gelu__prompt_kernel(
    A_x, A_mem0, A_Wq, A_Wk, A_Wv, A_Wo, A_seg_len, B_x, B_w1, B_b1, B_w2, B_b2, c, w_mod,
):
    del B_x
    assert A_x.shape == (1, S, DM) and int(A_seg_len) == SEG
    hbm = pl.BlockSpec(memory_space=pl.ANY)
    vmem = pl.BlockSpec(memory_space=pltpu.VMEM)
    out = pl.pallas_call(
        _kernel,
        out_shape=jax.ShapeDtypeStruct((S, DM), BF16),
        in_specs=[hbm, vmem, hbm, hbm, hbm, hbm, hbm, vmem, hbm, vmem, vmem, hbm],
        out_specs=hbm,
        scratch_shapes=[
            pltpu.VMEM((3 * H, DM // 2, DH), U32),
            pltpu.VMEM((H * DH // 2, DM), U32),
            pltpu.VMEM((DM // 2, FF), U32),
            pltpu.VMEM((FF // 2, DM), U32),
            pltpu.VMEM((S + 32, DM), BF16),
            pltpu.VMEM((S, DM), BF16),
            pltpu.VMEM((3 * H, RING, DH), F32),
            pltpu.VMEM((RING, H * DH), F32),
            pltpu.VMEM((BLK, DM), F32),
            pltpu.VMEM((BLK, DM), F32),
            pltpu.VMEM((BLK, FF), BF16),
            pltpu.VMEM((8, 6 * DM), F32),
            pltpu.VMEM((2, DM, HC // 2, DH), U32),
            pltpu.VMEM((2, DM, DM), BF16),
            pltpu.SemaphoreType.DMA((11,)),
        ],
        compiler_params=pltpu.CompilerParams(vmem_limit_bytes=124 * 1024 * 1024),
    )(A_x.reshape(S, DM), A_mem0.reshape(M, DM), A_Wq, A_Wk, A_Wv, A_Wo.reshape(H * DH, DM),
      B_w1, B_b1.reshape(1, FF), B_w2, B_b2.reshape(1, DM), c, w_mod)
    return out.reshape(1, S, DM)
```

```python
import functools

import jax
import jax.numpy as jnp
import numpy as np
from jax import lax
import jax.experimental.pallas as pl
import jax.experimental.pallas.tpu as pltpu

S, DM, H, DH, M, SEG, FF = 2048, 1024, 32, 128, 8, 32, 3584
NSEG = S // SEG
TOK = 24
TAILN = S - NSEG * TOK
LEAD = TAILN + 32
RING = 576
ROFF = (-LEAD) % TOK
NIT = NSEG // 2
BLK = 2 * TOK
HC = 16
EPS = 1e-5
F32, BF16, U32 = jnp.float32, jnp.bfloat16, jnp.uint32


def _ln_mod(x, scale, shift):
    m = jnp.mean(x, axis=-1, keepdims=True)
    xc = x - m
    v = jnp.mean(xc * xc, axis=-1, keepdims=True)
    return xc * lax.rsqrt(v + EPS) * (1.0 + scale) + shift


def _gelu(x):
    c = float(np.sqrt(2.0 / np.pi))
    return 0.5 * x * (1.0 + jnp.tanh(c * (x + 0.044715 * (x * x * x))))


def _w(ref_val):
    return pltpu.bitcast(ref_val, BF16)


def _dot(a, b):
    return jnp.dot(a, b, preferred_element_type=F32)


def _kernel(x_hbm, mem0_ref, wq_hbm, wk_hbm, wv_hbm, wo_hbm, w1_hbm, b1_ref, w2_hbm, b2_ref,
            c_ref, wmod_hbm, out_hbm,
            wqkv, wo, w1, w2, xs, outs, ring, oring, x1buf, hxbuf, ubuf, mod, stage, mstage, sems):
    NCH = 3 * (H // HC)
    w_src = (wq_hbm.bitcast(U32), wk_hbm.bitcast(U32), wv_hbm.bitcast(U32))

    def qkv_copy(c):
        m, g = divmod(c, H // HC)
        return pltpu.make_async_copy(w_src[m].at[:, pl.ds(g * (HC // 2), HC // 2), :],
                                     stage.at[c % 2], sems.at[c % 2])

    def mod_copy(j):
        return pltpu.make_async_copy(wmod_hbm.at[:, pl.ds(j * DM, DM)], mstage.at[j % 2],
                                     sems.at[2 + j % 2])

    x_copy0 = pltpu.make_async_copy(x_hbm.at[pl.ds(0, LEAD)], xs.at[pl.ds(0, LEAD)], sems.at[4])
    x_copy1 = pltpu.make_async_copy(x_hbm.at[pl.ds(LEAD, S - LEAD)], xs.at[pl.ds(LEAD, S - LEAD)],
                                    sems.at[5])
    wo_copy = pltpu.make_async_copy(wo_hbm.bitcast(U32), wo, sems.at[6])
    w1_copy = pltpu.make_async_copy(w1_hbm.bitcast(U32), w1, sems.at[7])
    w2_copy = pltpu.make_async_copy(w2_hbm.bitcast(U32), w2, sems.at[8])

    cv = c_ref[...].astype(F32)
    sc = jnp.broadcast_to(cv * jax.nn.sigmoid(cv), (16, DM)).astype(BF16)

    def mod_chunk(j):
        mod_copy(j).wait()
        mod[:, pl.ds(j * DM, DM)] = _dot(sc, mstage[j % 2])[:8]

    xs[pl.ds(S, 32), :] = jnp.zeros((32, DM), BF16)
    def relayout(c):
        qkv_copy(c).wait()
        st = stage.at[c % 2].reshape(DM * HC // 2, DH)
        for j in range(HC // 2):
            a = st[pl.ds(j, DM // 2, stride=HC), :]
            b = st[pl.ds(HC // 2 + j, DM // 2, stride=HC), :]
            wqkv[c * HC + 2 * j] = (a & U32(0xFFFF)) | (b << 16)
            wqkv[c * HC + 2 * j + 1] = (a >> 16) | (b & U32(0xFFFF0000))
        if c + 2 < NCH:
            qkv_copy(c + 2).start()

    qkv_copy(0).start()
    mod_copy(0).start()
    mod_copy(1).start()
    x_copy0.start()
    qkv_copy(1).start()
    relayout(0)
    mod_chunk(0)
    mod_chunk(1)
    x_copy0.wait()
    mod_copy(2).start()

    sa, ca = mod[0:1, 0:DM], mod[0:1, DM:2 * DM]
    h0buf = outs.at[pl.ds(0, LEAD)]
    h0buf[...] = _ln_mod(xs[0:LEAD].astype(F32), ca, sa).astype(BF16)
    for c in range(NCH):
        if c == 0:
            wo_copy.start()
        elif c == 2:
            mod_chunk(2)
            mod_copy(3).start()
            mod_copy(4).start()
        elif c == 3:
            x_copy1.start()
            w1_copy.start()
        elif c == 4:
            mod_chunk(3)
            mod_copy(5).start()
            mod_chunk(4)
            w2_copy.start()

        for t in range(c * HC, (c + 1) * HC):
            ring[t, pl.ds(ROFF, LEAD), :] = _dot(h0buf[...], _w(wqkv[t]))
            if t == c * HC + HC // 2 and c + 1 < NCH:
                relayout(c + 1)
    mod_chunk(5)
    wo_copy.wait()
    x_copy1.wait()

    ga = mod[0:1, 2 * DM:3 * DM]
    sb, cb, gb = mod[0:1, 3 * DM:4 * DM], mod[0:1, 4 * DM:5 * DM], mod[0:1, 5 * DM:6 * DM]
    b1 = b1_ref[...].astype(F32)
    b2 = b2_ref[...].astype(F32)

    def ffn(x1):
        h2 = _ln_mod(x1, cb, sb).astype(BF16)
        u = _gelu(_dot(h2, _w(w1[...])) + b1).astype(BF16)
        return (x1 + gb * (_dot(u, _w(w2[...])) + b2)).astype(BF16)

    L = M + SEG
    row = lax.broadcasted_iota(jnp.int32, (L, DH), 0)
    col = lax.broadcasted_iota(jnp.int32, (L, DH), 1)
    mask = (col < L) & ((row < M) | (row >= col))
    zpad = jnp.zeros((DH - L, DH), F32)
    scale = float(DH) ** -0.5

    G = 8

    def step(s, mem, hx, fill):
        lhs = jnp.concatenate([mem, hx], axis=0).astype(BF16)
        wslot = pl.multiple_of((LEAD + ROFF + TOK * s) % RING, 8)
        rs = [pl.multiple_of((SEG * s + ROFF + 8 * q) % RING, 8) for q in range(4)]
        oslot = pl.multiple_of((SEG * s) % RING, 32)
        rslot = pl.multiple_of((TOK * s) % RING, 8)
        mrow, lhs2, acc, tokr = {}, {}, {}, {}

        def proj(t):
            r = _dot(lhs, _w(wqkv[t]))
            tokr[t] = r[M:]
            mrow[t] = r[:M]

        def ext(t, pad):
            parts = [mrow[t]] + [ring[t, pl.ds(r, 8), :] for r in rs]
            return jnp.concatenate(parts + [zpad] * pad, axis=0)

        def attend(h):
            q = (ext(h, 0) * scale).astype(BF16)
            k = ext(H + h, 1).astype(BF16)
            sc_ = lax.dot_general(q, k, (((1,), (1,)), ((), ())), preferred_element_type=F32)
            sc_ = jnp.where(mask, sc_, -1e9)
            p = jnp.exp(sc_ - jnp.max(sc_, axis=-1, keepdims=True))
            l = jnp.sum(p, axis=-1, keepdims=True)
            r = pl.reciprocal(l, approx=True)
            r = r * (2.0 - l * r)
            o = _dot((p * r).astype(BF16), ext(2 * H + h, 1).astype(BF16))
            cs = pl.ds(h * DH, DH)
            oring[pl.ds(oslot, SEG), cs] = o[M:]
            lhs2[h] = jnp.concatenate([o[:M], oring[pl.ds(rslot, TOK), cs]], axis=0).astype(BF16)

        def outp(g, n):
            a = jnp.concatenate([lhs2[h] for h in range(g * G, (g + 1) * G)], axis=1)
            d = _dot(a, _w(wo[pl.ds(g * G * DH // 2, G * DH // 2), pl.ds(n * 128, 128)]))
            acc[n] = d if g == 0 else acc[n] + d

        NG = H // G
        for g in range(NG + 2):
            for j in range(G):
                if g < NG:
                    for m in range(3):
                        proj(m * H + g * G + j)
                if 1 <= g <= NG:
                    attend((g - 1) * G + j)
                if g >= 2:
                    outp(g - 2, j)
                    for m in range(3):
                        t = m * H + (g - 2) * G + j
                        ring[t, pl.ds(wslot, TOK), :] = tokr[t]
                if g >= NG:
                    for _ in range(2):
                        if fill:
                            fill.pop(0)()
        r2 = jnp.concatenate([acc[n] for n in range(DM // 128)], axis=1)
        return r2[:M], r2[M:]

    def ln_block(i):
        r = pl.multiple_of(jnp.minimum(LEAD + BLK * i, S + 32 - BLK), 16)
        hxbuf[...] = _ln_mod(xs[pl.ds(r, BLK), :].astype(F32), ca, sa)

    x1buf[...] = jnp.zeros((BLK, DM), F32)
    ln_block(0)
    NU, KP = FF // 128, 4
    KC = FF // KP

    def body(i, mem, ffn_on=True):
        x1 = x1buf[...]
        h2 = _ln_mod(x1, cb, sb).astype(BF16)
        prev = pl.multiple_of(jnp.maximum(BLK * (i - 1), 0), 16)
        acc = {}

        def up(n):
            cs = pl.ds(n * 128, 128)
            ubuf[:, cs] = _gelu(_dot(h2, _w(w1[:, cs])) + b1[:, n * 128:(n + 1) * 128]).astype(BF16)

        def down(n, k):
            cs = pl.ds(n * 128, 128)
            d = _dot(ubuf[:, pl.ds(k * KC, KC)], _w(w2[pl.ds(k * KC // 2, KC // 2), cs]))
            acc[n] = d if k == 0 else acc[n] + d
            if k == KP - 1:
                sl = slice(n * 128, (n + 1) * 128)
                outs[pl.ds(prev, BLK), cs] = (x1[:, sl] + gb[:, sl] * (acc[n] + b2[:, sl])).astype(BF16)

        ups = [functools.partial(up, n) for n in range(NU)]
        downs = [functools.partial(down, n, k) for n in range(DM // 128) for k in range(KP)]
        if not ffn_on:
            ups, downs = [], []
        mem, ya = step(2 * i, mem, hxbuf[0:TOK, :], ups)
        for f in downs[:8]:
            f()
        mem, yb = step(2 * i + 1, mem, hxbuf[TOK:BLK, :], downs[8:24] + [functools.partial(ln_block, i + 1)])
        for f in downs[24:]:
            f()
        xr = xs[pl.ds(pl.multiple_of(BLK * i, 16), BLK), :].astype(F32)
        x1buf[...] = xr + ga * jnp.concatenate([ya, yb], axis=0)
        return mem

    mem1 = body(0, mem0_ref[...].astype(F32), ffn_on=False)
    w1_copy.wait()
    w2_copy.wait()
    lax.fori_loop(1, NIT, body, mem1)

    DONE = BLK * (NIT - 1)
    out_copy0 = pltpu.make_async_copy(outs.at[pl.ds(0, DONE)], out_hbm.at[pl.ds(0, DONE)], sems.at[9])
    out_copy0.start()
    outs[pl.ds(DONE, BLK), :] = ffn(x1buf[...])
    EB = 256

    def tail(e, carry):
        p0 = NSEG * TOK + e * EB
        o = jnp.concatenate([oring[pl.ds((p0 + 64 * q) % RING, 64), :]
                             for q in range(EB // 64)], axis=0)
        y = _dot(o.astype(BF16), _w(wo[...]))
        x1 = xs[pl.ds(p0, EB), :].astype(F32) + ga * y
        outs[pl.ds(p0, EB), :] = ffn(x1)
        return carry

    for e in range(TAILN // EB):
        tail(e, 0)
    out_copy1 = pltpu.make_async_copy(outs.at[pl.ds(DONE, S - DONE)], out_hbm.at[pl.ds(DONE, S - DONE)],
                                      sems.at[10])
    out_copy1.start()
    out_copy0.wait()
    out_copy1.wait()


@functools.partial(jax.jit, static_argnames=("A_seg_len",))
def pallas_adaLN_cond__memory_aug_recurrent_mem_tr__dense_activation_gelu__prompt_kernel(
    A_x, A_mem0, A_Wq, A_Wk, A_Wv, A_Wo, A_seg_len, B_x, B_w1, B_b1, B_w2, B_b2, c, w_mod,
):
    del B_x
    assert A_x.shape == (1, S, DM) and int(A_seg_len) == SEG
    hbm = pl.BlockSpec(memory_space=pl.ANY)
    vmem = pl.BlockSpec(memory_space=pltpu.VMEM)
    out = pl.pallas_call(
        _kernel,
        out_shape=jax.ShapeDtypeStruct((S, DM), BF16),
        in_specs=[hbm, vmem, hbm, hbm, hbm, hbm, hbm, vmem, hbm, vmem, vmem, hbm],
        out_specs=hbm,
        scratch_shapes=[
            pltpu.VMEM((3 * H, DM // 2, DH), U32),
            pltpu.VMEM((H * DH // 2, DM), U32),
            pltpu.VMEM((DM // 2, FF), U32),
            pltpu.VMEM((FF // 2, DM), U32),
            pltpu.VMEM((S + 32, DM), BF16),
            pltpu.VMEM((S, DM), BF16),
            pltpu.VMEM((3 * H, RING, DH), F32),
            pltpu.VMEM((RING, H * DH), F32),
            pltpu.VMEM((BLK, DM), F32),
            pltpu.VMEM((BLK, DM), F32),
            pltpu.VMEM((BLK, FF), BF16),
            pltpu.VMEM((8, 6 * DM), F32),
            pltpu.VMEM((2, DM, HC // 2, DH), U32),
            pltpu.VMEM((2, DM, DM), BF16),
            pltpu.SemaphoreType.DMA((11,)),
        ],
        compiler_params=pltpu.CompilerParams(vmem_limit_bytes=124 * 1024 * 1024),
    )(A_x.reshape(S, DM), A_mem0.reshape(M, DM), A_Wq, A_Wk, A_Wv, A_Wo.reshape(H * DH, DM),
      B_w1, B_b1.reshape(1, FF), B_w2, B_b2.reshape(1, DM), c, w_mod)
    return out.reshape(1, S, DM)
```
